```python
import jax
import jax.numpy as jnp

def _softmax(x, axis=-1):
    return jax.nn.softmax(x, axis=axis)
def _gelu(x):
    return jax.nn.gelu(x, approximate=True)
def _silu(x):
    return jax.nn.silu(x)
def _sigmoid(x):
    return jax.nn.sigmoid(x)
def _layernorm(x, axis=-1, eps=1e-5):
    m = jnp.mean(x, axis=axis, keepdims=True)
    v = jnp.var(x, axis=axis, keepdims=True)
    return (x - m) / jnp.sqrt(v + eps)
def _scatter_add(tgt, idx, src, axis=0):
    return tgt.at[idx].add(src)
def _segment_sum(src, seg, n):
    return jax.ops.segment_sum(src, seg, n)
class _Rng:
    def __init__(self, key):
        self._k = key
    def _next(self):
        self._k, sub = jax.random.split(self._k)
        return sub
    def normal(self, shape):
        return jax.random.normal(self._next(), shape, dtype=jnp.bfloat16)
    def randint(self, lo, hi, shape):
        return jax.random.randint(self._next(), shape, lo, hi, dtype=jnp.int32)
    def uniform(self, shape, lo=0.0, hi=1.0):
        return jax.random.uniform(self._next(), shape, jnp.bfloat16, lo, hi)
    def permutation(self, n):
        return jax.random.permutation(self._next(), n)


kernel_name = 'parallel_sum__gqa_block_cached__moe_arch_mod__decode'

def setup_inputs():
    _rng = _Rng(jax.random.key(int.from_bytes(__import__("os").urandom(4), "little")))
    _w = (lambda a: (lambda t: t.astype(jnp.bfloat16) if jnp.issubdtype(t.dtype, jnp.floating) else t)(jnp.asarray(a)))
    def _A_setup():
        B, Sq, D = 1, 1, 448
        Hq, Hkv, Sk, Dh = 16, 8, 65536, 256
        assert Hq % Hkv == 0, (Hq, Hkv)
        return {
            "x": _w((lambda *s: _rng.normal(s) * 0.05)(B, Sq, D)),
            "k_cache": _w((lambda *s: _rng.normal(s) * 0.05)(B, Hkv, Sk, Dh)),
            "v_cache": _w((lambda *s: _rng.normal(s) * 0.05)(B, Hkv, Sk, Dh)),
            "wq": _w((lambda *s: _rng.normal(s) * 0.05)(D, Hq * Dh) * (D ** -0.5)),
            "wo": _w((lambda *s: _rng.normal(s) * 0.05)(Hq * Dh, D) * ((Hq * Dh) ** -0.5)),
        }
    _A_in = _A_setup()

    def _B_setup():
        B, S, D, F, C = 1, 1, 448, 1792, 1
        return {
            "x": _w((lambda *s: _rng.normal(s) * 0.05)(B, S, D)),
            "w_r": _w((lambda *s: _rng.normal(s) * 0.05)(D)),
            "w_gate": _w((lambda *s: _rng.normal(s) * 0.05)(D, F)),
            "w_up": _w((lambda *s: _rng.normal(s) * 0.05)(D, F)),
            "w_down": _w((lambda *s: _rng.normal(s) * 0.05)(F, D)),
        }
    _B_in = _B_setup()

    return {
        "A_x": _A_in["x"],
        "A_k_cache": _A_in["k_cache"],
        "A_v_cache": _A_in["v_cache"],
        "A_wq": _A_in["wq"],
        "A_wo": _A_in["wo"],
        "B_x": _B_in["x"],
        "B_w_r": _B_in["w_r"],
        "B_w_gate": _B_in["w_gate"],
        "B_w_up": _B_in["w_up"],
        "B_w_down": _B_in["w_down"],
    }

def reference(A_x, A_k_cache, A_v_cache, A_wq, A_wo, B_x, B_w_r, B_w_gate, B_w_up, B_w_down):
    def _A_ref(x, k_cache, v_cache, wq, wo):
        B, Sq, D = x.shape
        Hq, Dh = 16, 256
        Hkv = k_cache.shape[1]
        rep = Hq // Hkv
        q = (lambda x, *d: x.transpose(*d))((x @ wq).reshape(B, Sq, Hq, Dh), 0, 2, 1, 3)
        k = jnp.repeat(k_cache, rep, axis=1)
        v = jnp.repeat(v_cache, rep, axis=1)
        scores = jnp.einsum("bhqd,bhkd->bhqk", q, k) * (Dh ** -0.5)
        p = _softmax(scores, axis=-1)
        o = jnp.einsum("bhqk,bhkd->bhqd", p, v)
        return (lambda x, *d: x.transpose(*d))(o, 0, 2, 1, 3).reshape(B, Sq, Hq * Dh) @ wo

    def _B_ref(x, w_r, w_gate, w_up, w_down):
        B, S, D = x.shape
        C = 1
        r = x @ w_r
        idx = jnp.argsort(-r, axis=-1)[:, :C]
        idx_e = jnp.repeat(idx.reshape(B, C, 1), D, axis=2)
        x_sel = jnp.take_along_axis(x, idx_e, axis=1)
        g = _silu(x_sel @ w_gate)
        u = x_sel @ w_up
        y = (g * u) @ w_down
        r_sel = _sigmoid(jnp.take_along_axis(r, idx, axis=1))
        y = y * r_sel.reshape(B, C, 1)
        b_off = (jnp.arange(B) * S).reshape(B, 1)
        flat_idx = (idx + b_off).reshape(B * C)
        zero = (x * 0.0).reshape(B * S, D)
        upd = _scatter_add(zero, flat_idx, y.reshape(B * C, D), axis=0)
        return x + upd.reshape(B, S, D)

    x = A_x
    xn = _layernorm(x, axis=-1)
    return x + _A_ref(xn, A_k_cache, A_v_cache, A_wq, A_wo) + _B_ref(xn, B_w_r, B_w_gate, B_w_up, B_w_down)
```

```python
import functools
import jax, jax.numpy as jnp
from jax.experimental import pallas as pl
from jax.experimental.pallas import tpu as pltpu

D, F, HKV, SK, DH = 448, 1792, 8, 65536, 256
f32, bf16 = jnp.float32, jnp.bfloat16
NT = (((1,), (1,)), ((), ()))

def chunks(n, rows):
    out = []; o = 0
    while o < n:
        r = min(rows, n - o); out.append((o, r)); o += r
    return out

def pat_gen(sb, rows, ns, g, pm, order):
    part = sb // ns; ch = chunks(part, rows); out = []; t = 0
    for i in range(0, len(ch), g):
        seq = [(a, j) for a in (0, 1) for j in range(ns)] if order == 'av' else [(a, j) for j in range(ns) for a in (0, 1)]
        for a, j in seq:
            for o, r in ch[i:i + g]:
                p = {'alt': t % 2, 'arr': a, 'str': j % 2}[pm]
                out.append((a, j * part + o, r, p)); t += 1
    return out

def make(sb=2048, nbuf=4, pattern=None, cs=None, wrows=8, ffn_head=1, bounds=False):
    pattern = pattern or pat_gen(sb, 80, 1, 2, 'alt', 'av')
    cs = cs or sb
    nb = SK // sb
    n = HKV * nb

    def kern(x_hbm, wr_hbm, k_hbm, v_hbm, wq_hbm, wot_hbm, wg_hbm, wu_hbm, wdt_hbm, o_ref,
             xb, wrb, wqb, wob, wgb, wub, wdb, qs, kv, sem, wsem):
        def start_kv(i, s):
            for a, o, r, p in pattern:
                src = (k_hbm, v_hbm)[a]
                pltpu.make_async_copy(src.at[pl.ds(pl.multiple_of(i * sb + o, 8), r)],
                                      kv.at[s, a, pl.ds(o, r)], sem.at[s]).start(priority=p)
        def wait_kv(s):
            pltpu.make_async_copy(kv.at[s], kv.at[s], sem.at[s]).wait()
        def start_w(src, dst, j, rows):
            for t, (o, r) in enumerate(chunks(D, rows)):
                pltpu.make_async_copy(src.at[pl.ds(o, r)], dst.at[pl.ds(o, r)], wsem.at[j]).start(priority=t % 2)
        def wait_w(dst, j):
            pltpu.make_async_copy(dst, dst, wsem.at[j]).wait()

        cx = pltpu.make_async_copy(x_hbm, xb, wsem.at[0]); cx.start()
        cr = pltpu.make_async_copy(wr_hbm, wrb, wsem.at[1]); cr.start(priority=1)
        start_w(wq_hbm, wqb, 2, wrows)
        for i in range(nbuf - 1):
            start_kv(i, i)
        cx.wait(); cr.wait()
        x = xb[0].astype(f32)
        mu = jnp.mean(x, axis=-1, keepdims=True)
        xc = x - mu
        var = jnp.mean(xc * xc, axis=-1, keepdims=True)
        xn = (xc * jax.lax.rsqrt(var + 1e-5)).astype(bf16)
        xnf = xn.astype(f32)
        x8 = jnp.broadcast_to(xn, (8, D))
        r = jnp.sum(xnf * wrb[...].astype(f32).reshape(1, D), axis=-1, keepdims=True)
        gate = jax.nn.sigmoid(r.astype(bf16).astype(f32))
        wait_w(wqb, 2)
        odd = (jax.lax.broadcasted_iota(jnp.int32, (8, DH), 0) % 2) == 1
        for h in range(HKV):
            q = jnp.dot(x8, wqb[:, h * 512:(h + 1) * 512], preferred_element_type=f32)
            q = q.astype(bf16).astype(f32) * (DH ** -0.5)
            qs[h] = jnp.where(odd, q[:, DH:], q[:, :DH]).astype(bf16)

        y = jnp.zeros((8, D), f32)
        yb = None
        for h in range(HKV):
            if h == ffn_head:
                start_w(wg_hbm, wgb, 3, 2 * wrows); start_w(wu_hbm, wub, 4, 2 * wrows); start_w(wdt_hbm, wdb, 5, 2 * wrows)
            if h == 0:
                start_w(wot_hbm, wob, 6, wrows)
            qh = qs[h]
            def body(j, c, h=h, qh=qh):
                m, l, acc = c
                i = h * nb + j
                s = i % nbuf
                wait_kv(s)
                nx = i + nbuf - 1
                if h == HKV - 1:
                    @pl.when(nx < n)
                    def _(): start_kv(nx, nx % nbuf)
                else:
                    start_kv(nx, nx % nbuf)
                for c0 in range(0, sb, cs):
                    sc = jax.lax.dot_general(qh, kv[s, 0, c0:c0 + cs, :], NT, preferred_element_type=f32)
                    mn = jnp.maximum(m, jnp.max(sc, axis=-1, keepdims=True))
                    al = jnp.exp(m - mn)
                    p = jnp.exp(sc - mn)
                    ps = p[:, 0:128]
                    for t in range(128, cs, 128):
                        ps = ps + p[:, t:t + 128]
                    l = l * al + ps
                    acc = acc * al + jnp.dot(p.astype(bf16), kv[s, 1, c0:c0 + cs, :], preferred_element_type=f32)
                    m = mn
                return m, l, acc
            m, l, acc = jax.lax.fori_loop(0, nb, body, (jnp.full((8, 1), -jnp.inf, f32), jnp.zeros((8, 128), f32), jnp.zeros((8, DH), f32)))
            o = (acc / jnp.sum(l, axis=-1, keepdims=True)).astype(bf16)
            z = jnp.zeros_like(o)
            oc = jnp.concatenate([jnp.where(odd, z, o), jnp.where(odd, o, z)], axis=1)
            if h == 0:
                wait_w(wob, 6)
            y = y + jax.lax.dot_general(oc, wob[:, h * 512:(h + 1) * 512], NT, preferred_element_type=f32)
            if h == ffn_head:
                wait_w(wgb, 3); wait_w(wub, 4); wait_w(wdb, 5)
                g = jnp.dot(x8, wgb[...], preferred_element_type=f32)
                u = jnp.dot(x8, wub[...], preferred_element_type=f32)
                hh = (g * jax.nn.sigmoid(g) * u).astype(bf16)
                yb = jax.lax.dot_general(hh, wdb[...], NT, preferred_element_type=f32)[0:1] * gate
        res = x + (y[0:1] + y[1:2]) + (xnf + yb)
        o_ref[0] = res.astype(bf16)

    def fn(A_x, A_k_cache, A_v_cache, A_wq, A_wo, B_x, B_w_r, B_w_gate, B_w_up, B_w_down):
        k = A_k_cache.reshape(HKV * SK, DH); v = A_v_cache.reshape(HKV * SK, DH)
        return pl.pallas_call(kern, out_shape=jax.ShapeDtypeStruct((1, 1, D), bf16),
            in_specs=[pl.BlockSpec(memory_space=pl.ANY)] * 9,
            scratch_shapes=[pltpu.VMEM((1, 1, D), bf16), pltpu.VMEM((D,), bf16),
                            pltpu.VMEM((D, 4096), bf16), pltpu.VMEM((D, 4096), bf16),
                            pltpu.VMEM((D, F), bf16), pltpu.VMEM((D, F), bf16), pltpu.VMEM((D, F), bf16),
                            pltpu.VMEM((HKV, 8, DH), bf16),
                            pltpu.VMEM((nbuf, 2, sb, DH), bf16),
                            pltpu.SemaphoreType.DMA((nbuf,)), pltpu.SemaphoreType.DMA((7,))],
            compiler_params=pltpu.CompilerParams(vmem_limit_bytes=100 * 2**20, disable_bounds_checks=not bounds),
        )(A_x, B_w_r, k, v, A_wq, A_wo.T, B_w_gate, B_w_up, B_w_down.T)
    return fn


_fn = make(4096,3)


@jax.jit
def pallas_parallel_sum__gqa_block_cached__moe_arch_mod__decode_kernel(
    A_x, A_k_cache, A_v_cache, A_wq, A_wo, B_x, B_w_r, B_w_gate, B_w_up, B_w_down,
):
    return _fn(A_x, A_k_cache, A_v_cache, A_wq, A_wo, B_x, B_w_r, B_w_gate, B_w_up, B_w_down)
```

```python
import jax
import jax.numpy as jnp
from jax.experimental import pallas as pl
from jax.experimental.pallas import tpu as pltpu

D, F, HKV, SK, DH = 448, 1792, 8, 65536, 256
HW = 2 * DH
f32, bf16 = jnp.float32, jnp.bfloat16
NT = (((1,), (1,)), ((), ()))


def even_cuts(part, rows):
    n8, k = part // 8, round(part / rows)
    e = [(t * n8) // k * 8 for t in range(k + 1)]
    return [(a, b - a) for a, b in zip(e, e[1:])]


def make(sb=4096, nbuf=2, ns=4, nst=4, look=5, cuts=None, kperm=None, vperm=None, ffn_head=1, swap=0):
    part = sb // ns
    st_rows = part // nst
    cuts = cuts or even_cuts(part, 72)
    kperm = kperm or list(range(ns))
    vperm = vperm or kperm
    nb = SK // sb
    n = HKV * nb
    assert look <= nbuf * nst - 2

    def kern(x_hbm, wr_hbm, k_hbm, v_hbm, wq_hbm, wot_hbm, wg_hbm, wu_hbm, wdt_hbm, o_ref,
             xb, wrb, wqb, wob, wgb, wub, wdb, qs, kv, sem, wsem):
        def kv_copies(i, st):
            s = i % nbuf
            out = []
            for o, r in cuts:
                if o // st_rows != st:
                    continue
                for js in zip(kperm, vperm):
                    for a, src in enumerate((k_hbm, v_hbm)):
                        c = js[a] * part + o
                        out.append((a ^ swap, pltpu.make_async_copy(
                            src.at[pl.ds(pl.multiple_of(i * sb + c, 8), r)],
                            kv.at[s, a, pl.ds(c, r)], sem.at[s, st])))
            return out

        def start_kv(i, st):
            for p, c in kv_copies(i, st):
                c.start(priority=p)

        def wait_kv(i, st):
            for _, c in kv_copies(i, st):
                c.wait()

        def start_w(src, dst, j):
            half = src.shape[1] // 2
            for o0 in range(0, D // 4, 8):
                for o in range(o0, D, D // 4):
                    for p in range(2):
                        ix = (pl.ds(o, 8), pl.ds(p * half, half))
                        pltpu.make_async_copy(src.at[ix], dst.at[ix], wsem.at[j]).start(priority=p)

        def wait_w(dst, j):
            pltpu.make_async_copy(dst, dst, wsem.at[j]).wait()

        cx = pltpu.make_async_copy(x_hbm, xb, wsem.at[0])
        cr = pltpu.make_async_copy(wr_hbm, wrb, wsem.at[1])
        cx.start()
        cr.start(priority=1)
        start_w(wq_hbm, wqb, 2)
        for u in range(look):
            start_kv(u // nst, u % nst)
        cx.wait()
        cr.wait()

        x = xb[0].astype(f32)
        xc = x - jnp.mean(x, axis=-1, keepdims=True)
        var = jnp.mean(xc * xc, axis=-1, keepdims=True)
        xn = (xc * jax.lax.rsqrt(var + 1e-5)).astype(bf16)
        xnf = xn.astype(f32)
        x8 = jnp.broadcast_to(xn, (8, D))
        r = jnp.sum(xnf * wrb[...].astype(f32).reshape(1, D), axis=-1, keepdims=True)
        gate = jax.nn.sigmoid(r)

        odd = (jax.lax.broadcasted_iota(jnp.int32, (8, DH), 0) % 2) == 1
        wait_w(wqb, 2)
        for h in range(HKV):
            q = jnp.dot(x8, wqb[:, h * HW:(h + 1) * HW], preferred_element_type=f32) * (DH ** -0.5)
            qs[h] = jnp.where(odd, q[:, DH:], q[:, :DH]).astype(bf16)

        ya = jnp.zeros((8, D), f32)
        yb = None
        for h in range(HKV):
            if h == 0:
                start_w(wot_hbm, wob, 3)
            if h == ffn_head:
                start_w(wg_hbm, wgb, 4)
                start_w(wu_hbm, wub, 5)
                start_w(wdt_hbm, wdb, 6)
            qh = qs[h]

            def body(j, carry, h=h, qh=qh):
                m, l, acc = carry
                i = h * nb + j
                s = i % nbuf
                for st in range(nst):
                    wait_kv(i, st)
                    nx = i + (st + look) // nst
                    if h == HKV - 1:
                        @pl.when(nx < n)
                        def _():
                            start_kv(nx, (st + look) % nst)
                    else:
                        start_kv(nx, (st + look) % nst)

                    def rows(a):
                        return jnp.concatenate(
                            [kv[s, a, pl.ds(t * part + st * st_rows, st_rows), :] for t in range(ns)], axis=0)
                    sc = jax.lax.dot_general(qh, rows(0), NT, preferred_element_type=f32)
                    mn = jnp.maximum(m, jnp.max(sc, axis=-1, keepdims=True))
                    al = jnp.exp(m - mn)
                    p = jnp.exp(sc - mn)
                    ps = p[:, 0:128]
                    for t in range(128, ns * st_rows, 128):
                        ps = ps + p[:, t:t + 128]
                    l = l * al + ps
                    acc = acc * al + jnp.dot(p.astype(bf16), rows(1), preferred_element_type=f32)
                    m = mn
                return m, l, acc

            init = (jnp.full((8, 1), -jnp.inf, f32), jnp.zeros((8, 128), f32), jnp.zeros((8, DH), f32))
            _, l, acc = jax.lax.fori_loop(0, nb, body, init)
            o = (acc / jnp.sum(l, axis=-1, keepdims=True)).astype(bf16)
            z = jnp.zeros_like(o)
            oc = jnp.concatenate([jnp.where(odd, z, o), jnp.where(odd, o, z)], axis=1)
            if h == 0:
                wait_w(wob, 3)
            ya = ya + jax.lax.dot_general(oc, wob[:, h * HW:(h + 1) * HW], NT, preferred_element_type=f32)
            if h == ffn_head:
                wait_w(wgb, 4)
                wait_w(wub, 5)
                wait_w(wdb, 6)
                g = jnp.dot(x8, wgb[...], preferred_element_type=f32)
                u = jnp.dot(x8, wub[...], preferred_element_type=f32)
                hh = (g * jax.nn.sigmoid(g) * u).astype(bf16)
                yb = jax.lax.dot_general(hh, wdb[...], NT, preferred_element_type=f32)[0:1] * gate
        o_ref[0] = (x + (ya[0:1] + ya[1:2]) + (xnf + yb)).astype(bf16)

    def fn(A_x, A_k_cache, A_v_cache, A_wq, A_wo, B_x, B_w_r, B_w_gate, B_w_up, B_w_down):
        del B_x
        return pl.pallas_call(
            kern,
            out_shape=jax.ShapeDtypeStruct((1, 1, D), bf16),
            in_specs=[pl.BlockSpec(memory_space=pl.ANY)] * 9,
            scratch_shapes=[
                pltpu.VMEM((1, 1, D), bf16), pltpu.VMEM((D,), bf16),
                pltpu.VMEM((D, HKV * HW), bf16), pltpu.VMEM((D, HKV * HW), bf16),
                pltpu.VMEM((D, F), bf16), pltpu.VMEM((D, F), bf16), pltpu.VMEM((D, F), bf16),
                pltpu.VMEM((HKV, 8, DH), bf16),
                pltpu.VMEM((nbuf, 2, sb, DH), bf16),
                pltpu.SemaphoreType.DMA((nbuf, nst)), pltpu.SemaphoreType.DMA((7,)),
            ],
            compiler_params=pltpu.CompilerParams(
                vmem_limit_bytes=64 * 2**20, disable_bounds_checks=True),
        )(A_x, B_w_r, A_k_cache.reshape(HKV * SK, DH), A_v_cache.reshape(HKV * SK, DH),
          A_wq, A_wo.T, B_w_gate, B_w_up, B_w_down.T)
    return fn


_fn = make(
    cuts=[(o + a, r) for o in range(0, 1024, 256) for a, r in ((0, 64), (64, 96), (160, 96))],
    kperm=[3, 1, 0, 2], vperm=[2, 0, 3, 1], swap=1)


@jax.jit
def pallas_parallel_sum__gqa_block_cached__moe_arch_mod__decode_kernel(
    A_x, A_k_cache, A_v_cache, A_wq, A_wo, B_x, B_w_r, B_w_gate, B_w_up, B_w_down,
):
    return _fn(A_x, A_k_cache, A_v_cache, A_wq, A_wo, B_x, B_w_r, B_w_gate, B_w_up, B_w_down)
```
